```python
import os as _os
_os.environ.setdefault("JAX_PLATFORMS", "cpu")
import jax
import jax.numpy as jnp

def _softmax(x, axis=-1):
    return jax.nn.softmax(x, axis=axis)
def _gelu(x):
    return jax.nn.gelu(x, approximate=True)
def _silu(x):
    return jax.nn.silu(x)
def _sigmoid(x):
    return jax.nn.sigmoid(x)
def _layernorm(x, axis=-1, eps=1e-5):
    m = jnp.mean(x, axis=axis, keepdims=True)
    v = jnp.var(x, axis=axis, keepdims=True)
    return (x - m) / jnp.sqrt(v + eps)
def _scatter_add(tgt, idx, src, axis=0):
    return tgt.at[idx].add(src)
def _segment_sum(src, seg, n):
    return jax.ops.segment_sum(src, seg, n)
class _Rng:
    def __init__(self, key):
        self._k = key
    def _next(self):
        self._k, sub = jax.random.split(self._k)
        return sub
    def normal(self, shape):
        return jax.random.normal(self._next(), shape, dtype=jnp.bfloat16)
    def randint(self, lo, hi, shape):
        return jax.random.randint(self._next(), shape, lo, hi, dtype=jnp.int32)
    def uniform(self, shape, lo=0.0, hi=1.0):
        return jax.random.uniform(self._next(), shape, jnp.bfloat16, lo, hi)
    def permutation(self, n):
        return jax.random.permutation(self._next(), n)


kernel_name = 'gated_mix__mha_block__ssm_conv_h3__prompt'

def setup_inputs():
    _rng = _Rng(jax.random.key(int.from_bytes(__import__("os").urandom(4), "little")))
    _w = (lambda a: (lambda t: t.astype(jnp.bfloat16) if jnp.issubdtype(t.dtype, jnp.floating) else t)(jnp.asarray(a)))
    def _A_setup():
        B, S, D, H = 1, 2048, 640, 32
        return {
            "x": _w((lambda *s: _rng.normal(s) * 0.05)(B, S, D)),
            "wqkv": _w((lambda *s: _rng.normal(s) * 0.4)(D, 3 * D)),
            "wo": _w((lambda *s: _rng.normal(s) * 0.05)(D, D)),
        }
    _A_in = _A_setup()

    def _B_setup():
        B, S, D = 1, 2048, 640
        ks = 4
        return {
            "q": _w((lambda *s: _rng.normal(s) * 0.05)(B, S, D)),
            "k": _w((lambda *s: _rng.normal(s) * 0.4)(B, S, D)),
            "v": _w((lambda *s: _rng.normal(s) * 0.4)(B, S, D)),
            "shift_k": _w((lambda *s: _rng.normal(s) * 0.4)(D, ks) * 0.5),
            "ssm_k": _w((lambda *s: _rng.normal(s) * 0.4)(D, S) * (1.0 / S ** 0.5)),
            "ssm_D": _w((lambda *s: _rng.normal(s) * 0.4)(D)),
        }
    _B_in = _B_setup()

    return {
        "A_x": _A_in["x"],
        "A_wqkv": _A_in["wqkv"],
        "A_wo": _A_in["wo"],
        "B_q": _B_in["q"],
        "B_k": _B_in["k"],
        "B_v": _B_in["v"],
        "B_shift_k": _B_in["shift_k"],
        "B_ssm_k": _B_in["ssm_k"],
        "B_ssm_D": _B_in["ssm_D"],
        "gate_w": _w((lambda *s: _rng.normal(s) * 0.05)(640) * 16.0),
    }

def reference(A_x, A_wqkv, A_wo, B_q, B_k, B_v, B_shift_k, B_ssm_k, B_ssm_D, gate_w):
    def _A_ref(x, wqkv, wo):
        B, S, D = x.shape
        H = 32
        Dh = D // H
        qkv = (lambda x, *d: x.transpose(*d))((x @ wqkv).reshape(B, S, 3, H, Dh), 2, 0, 3, 1, 4)
        q, k, v = qkv[0], qkv[1], qkv[2]
        scores = jnp.einsum("bhqd,bhkd->bhqk", q, k) * (Dh ** -0.5)
        p = _softmax(scores, axis=-1)
        o = jnp.einsum("bhqk,bhkd->bhqd", p, v)
        return (lambda x, *d: x.transpose(*d))(o, 0, 2, 1, 3).reshape(B, S, D) @ wo

    def _B_ref(q, k, v, shift_k, ssm_k, ssm_D):
        B, S, D = q.shape
        ks = shift_k.shape[-1]
        k_pad = jnp.pad(k, ((0, 0), (ks - 1, 0), (0, 0)))
        k_shift = jnp.zeros_like(k)
        for t in range(ks):
            k_shift = k_shift + k_pad[:, t:t + S, :] * shift_k[:, ks - 1 - t][None, None, :]
        kv = k_shift * v
        L = 2 * S
        kv_pad = jnp.pad(kv, ((0, 0), (0, S), (0, 0)))
        kf_pad = jnp.pad(ssm_k, ((0, 0), (0, S)))
        kv_f = (lambda x, axes=(-2,-1): jnp.fft.rfft2(x.astype(jnp.float32), axes=axes))(kv_pad[:, None, :, :], axes=(1, 2))
        kf_f = (lambda x, axes=(-2,-1): jnp.fft.rfft2(x.astype(jnp.float32), axes=axes))(kf_pad[:, None, :], axes=(1, 2))
        kf_f = (lambda x, *d: x.transpose(*d))(kf_f, 1, 2, 0)
        y_f = kv_f * kf_f[None, :, :, :]
        y = (lambda x, s, axes=(-2,-1): jnp.fft.irfft2(x, s=s, axes=axes).astype(jnp.bfloat16))(y_f, (1, L), axes=(1, 2))[:, 0, :S, :]
        y = y + kv * ssm_D[None, None, :]
        return q * y

    x = A_x
    g = _sigmoid((x * gate_w).sum(-1, keepdims=True))
    a = _A_ref(x, A_wqkv, A_wo)
    b = _B_ref(x, B_k, B_v, B_shift_k, B_ssm_k, B_ssm_D)
    return g * a + (1 - g) * b
```

```python
import functools

import jax
import jax.numpy as jnp
import numpy as np
from jax import lax
from jax.experimental import pallas as pl
from jax.experimental.pallas import tpu as pltpu

S, D, H = 2048, 640, 32
DH = D // H
NPAIR = H // 2
C = 128
NC = S // C
NL = D // 128
TQ = 512
F32, BF16, U32 = jnp.float32, jnp.bfloat16, jnp.uint32
QSCALE = float(DH ** -0.5 * np.log2(np.e))
L_LO, L_HI, O_HI = 2.0 ** -20, 2.0 ** 40, 2.0 ** 127

NN = (((1,), (0,)), ((), ()))
NT = (((1,), (1,)), ((), ()))
TN = (((0,), (0,)), ((), ()))


def _dft_tables():
    th = 2.0 * np.pi * (np.arange(C)[:, None] + 0.25) * np.arange(C)[None, :] / C
    fwd = np.concatenate([np.cos(th), -np.sin(th)], 0)
    inv = np.concatenate([np.cos(th).T, -np.sin(th).T], 0) / C
    ids = np.broadcast_to(np.ones((1, 1)), (8, C))
    return np.concatenate([fwd, inv, ids], 0).astype(np.float32)


_TABLES = _dft_tables()


def _dot(a, b, dims=NN):
    return lax.dot_general(a, b, dims, preferred_element_type=F32)


def _cat(xs, axis):
    return xs[0] if len(xs) == 1 else jnp.concatenate(xs, axis)


class _Pacer:
    def __init__(self, jobs, cycles, keep, lead=0):
        self.jobs, self.cycles, self.keep, self.lead = jobs, cycles, keep, lead
        self.total = sum(w for w, _ in jobs)
        self.t = self.done = self.i = 0

    def tie(self, x, dt):
        self.t += dt
        n = 0
        while self.i < len(self.jobs) and n < len(self.keep):
            w, job = self.jobs[self.i]
            if (self.done + w) * self.cycles > (self.t - self.lead) * self.total:
                break
            r = job()
            x = jnp.where(self.keep[n], x, r if r.dtype == x.dtype else pltpu.bitcast(r, x.dtype))
            self.done += w
            self.i += 1
            n += 1
        return x

    def flush(self):
        for _, job in self.jobs[self.i:]:
            job()
        self.i = len(self.jobs)


def build(nm=(112,) * 16, lead=48, tail=0, scopes=False, force_slow=False, mac_tie=True, qv_unroll=1,
          out_chunks=(512, 512, 512, 256, 256), x_chunks=(256, 256, 512, 512, 512), flags=None):
    vkeys = [(t, r) for t in range(NC) for r in range(nm[t], 128, 8)]
    vrow = {tr: 8 * i for i, tr in enumerate(vkeys)}
    nv = 8 * len(vkeys)

    def scope(name):
        import contextlib
        return jax.named_scope(name) if scopes else contextlib.nullcontext()

    def kernel(x_hbm, wqkv_hbm, wo_hbm, k_hbm, v_hbm, sk_hbm, h_hbm, d_hbm, g_hbm, tab_hbm, out_hbm,
               x_v, wq_v, wk_v, wv_v, wo_v, k_v, v_v, sk_v, h_v, d_v, g_v, tab_v, out_v,
               wt_s, kp_s, q_s, vt_s, ot_s, pa_s, pb_s, kv_s, uf_s, hf_s, yf_s, y_s, sems):
        sem_it = iter(range(32))

        def copy(src, dst):
            return pltpu.make_async_copy(src, dst, sems.at[next(sem_it)])

        xo = np.cumsum((0,) + tuple(x_chunks))
        cp_x = [copy(x_hbm.at[pl.ds(int(a), n)], x_v.at[pl.ds(int(a), n)]) for a, n in zip(xo, x_chunks)]
        cp_wk = copy(wqkv_hbm.at[:, pl.ds(D, D)], wk_v)
        cp_wq = copy(wqkv_hbm.at[:, pl.ds(0, D)], wq_v)
        cp_wv = copy(wqkv_hbm.at[:, pl.ds(2 * D, D)], wv_v)
        cp_wo, cp_k, cp_v, cp_h = copy(wo_hbm, wo_v), copy(k_hbm, k_v), copy(v_hbm, v_v), copy(h_hbm, h_v)
        cp_small = [copy(sk_hbm, sk_v), copy(d_hbm, d_v), copy(g_hbm, g_v), copy(tab_hbm, tab_v)]
        oo = np.cumsum((0,) + tuple(out_chunks))
        cp_o = [copy(out_v.at[pl.ds(int(a), n)], out_hbm.at[pl.ds(int(a), n)]) for a, n in zip(oo, out_chunks)]

        cp_wk.start()
        cp_x[0].start()
        cp_wk.wait()
        cp_x[0].wait()
        for c in cp_x[1:] + cp_small:
            c.start()
        later = [[], [cp_h], [cp_k], [cp_v], [cp_wq, cp_wv, cp_wo]]

        with scope("kproj"):
            for i, (a, n) in enumerate(zip(xo, x_chunks)):
                a = int(a)
                if i:
                    cp_x[i].wait()
                for c in later[i]:
                    c.start()
                kk = _dot(x_v[a:a + n, :], wk_v[...])
                low = lax.broadcasted_iota(jnp.int32, (n, 128), 1) < 64
                for p in range(NPAIR):
                    t, off = divmod(2 * DH * p, 128)
                    blk = kk[:, 128 * t:128 * (t + 1)]
                    if off + 2 * DH > 128:
                        blk = jnp.where(low, kk[:, 128 * (t + 1):128 * (t + 2)], blk)
                    kp_s[p, a:a + n, :] = pltpu.roll(blk, 128 - off, 1) if off else blk

        for c in cp_small:
            c.wait()

        def keeps():
            one = tab_v[4 * C:4 * C + 8, :]
            return [one > 0.25 * i for i in range(4)]

        with scope("dft"):
            cp_h.wait()
            fwd = tab_v[0:2 * C, :].astype(BF16)
            for c in range(NC):
                hf_s[c] = _dot(fwd, h_v[:, c * C:(c + 1) * C], NT)
            cp_k.wait()
            cp_v.wait()
            sk = sk_v[...].astype(F32)
            for c in range(NC):
                cur = k_v[c * C:(c + 1) * C, :].astype(F32)
                prev = k_v[c * C - 16:c * C, :].astype(F32)[8:] if c else jnp.zeros((8, D), F32)
                k0 = jnp.concatenate([prev, cur], 0)
                k1 = pltpu.roll(k0, 1, 0)
                far = pltpu.roll(k0 * sk[2:3] + k1 * sk[3:4], 2, 0)
                kv = (cur * sk[0:1] + k1[8:] * sk[1:2] + far[8:]) * v_v[c * C:(c + 1) * C, :].astype(F32)
                kv_s[c * C:(c + 1) * C, :] = kv
                uf_s[c] = _dot(fwd, kv)
            cp_wq.wait()
            cp_wv.wait()
            wt_s[0:D // 2, :] = pltpu.bitcast(wq_v[...].T, U32)
            wt_s[D // 2:D, :] = pltpu.bitcast(wv_v[...].T, U32)

        def mac_jobs(r0, l):
            st = {}
            cols = slice(128 * l, 128 * (l + 1))
            re, im = pl.ds(r0, 8), pl.ds(r0 + C, 8)

            def operands(which, c):
                if (which, c) not in st:
                    hr, hi = hf_s[c, re, cols], hf_s[c, im, cols]
                    if c:
                        hr, hi = hr - hf_s[c - 1, im, cols], hi + hf_s[c - 1, re, cols]
                    if which == 0:
                        st[which, c] = (hr, uf_s[c, re, cols] + uf_s[c, im, cols])
                    elif which == 1:
                        st[which, c] = (hi - hr, uf_s[c, re, cols])
                    else:
                        st[which, c] = (hi + hr, uf_s[c, im, cols])
                return st[which, c]

            def job(which, a):
                acc = None
                for b in range(a + 1):
                    t = operands(which, a - b)[0] * operands(which, b)[1]
                    acc = t if acc is None else acc + t
                if which == 0:
                    st[a] = acc
                elif which == 1:
                    acc = st[a] + acc
                    yf_s[a, im, cols] = acc
                else:
                    acc = st[a] - acc
                    yf_s[a, re, cols] = acc
                return acc

            return [(2 * a + 4, functools.partial(job, w, a)) for w in range(3) for a in range(NC)]

        def qv_body(i, _):
            jobs = []
            for u in range(qv_unroll):
                for r in range(4):
                    for l in range(NL):
                        jobs += mac_jobs(pl.multiple_of((i * qv_unroll + u) * 32 + r * 8, 8), l)
            pace = _Pacer(jobs, qv_unroll * 2 * D * NL, keeps(), lead)
            top = lax.broadcasted_iota(jnp.int32, (8, 128), 0) < 4
            for n in range(4 * qv_unroll):
                t0 = pl.multiple_of(i * qv_unroll * 512 + n * 128, 128)
                cols = []
                for kt in range(NL):
                    tied = mac_tie and (NL * n + kt) % 4 == 0
                    if tied:
                        w = _cat([pace.tie(wt_s[m:m + 8, 128 * kt:128 * (kt + 1)], 16) for m in range(0, D, 8)], 0)
                    else:
                        w = wt_s[:, 128 * kt:128 * (kt + 1)]
                    cols.append(w)
                r = _dot(pltpu.bitcast(_cat(cols, 1), BF16), x_v[pl.ds(t0, 128), :], NT)
                for ref, base, fill in ((q_s, 0, 0.0), (vt_s, D, 1.0)):
                    for p in range(NPAIR):
                        blk = r[base + 40 * p:base + 40 * (p + 1)]
                        if not base:
                            blk = blk * QSCALE
                        mid = blk[16:24]
                        ref[p, :, pl.ds(t0, 128)] = jnp.concatenate(
                            [blk[0:16], jnp.where(top, mid, fill), jnp.where(top, fill, mid), blk[24:40]], 0)
            pace.flush()

        with scope("qvproj"):
            lax.fori_loop(0, 4 // qv_unroll, qv_body, None)

        def score_jobs(p, odd, dst):
            st = {}

            def job(t, r, c):
                if (t, r) not in st:
                    kk = kp_s[p, 128 * t + r:128 * t + r + 8, :]
                    st.clear()
                    st[t, r] = [jnp.broadcast_to(kk[:, DH * odd + d:DH * odd + d + 1], (8, 128)) for d in range(DH)]
                acc = None
                for d in range(DH):
                    row = 28 * odd + d
                    term = st[t, r][d] * q_s[p, row:row + 1, 128 * c:128 * (c + 1)]
                    acc = term if acc is None else acc + term
                dst[vrow[t, r]:vrow[t, r] + 8, 128 * c:128 * (c + 1)] = jnp.exp2(acc)
                return acc

            return [(1, functools.partial(job, t, r, c)) for t, r in vkeys for c in range(S // 128)]

        with scope("idft"):
            pace = _Pacer(score_jobs(0, 0, pa_s), NC * NL * 2 * C // 4, keeps(), lead)
            inv = [pltpu.bitcast(tab_v[(2 + j) * C:(3 + j) * C, :].astype(BF16), U32) for j in range(2)]
            for c in range(NC):
                for l in range(NL):
                    left = inv[0]
                    if (c * NL + l) % 2 == 0:
                        left = _cat([pace.tie(left[m:m + 8], 16) for m in range(0, C // 2, 8)], 0)
                    lhs = pltpu.bitcast(jnp.concatenate([left, inv[1]], 1), BF16)
                    y_s[c * C:(c + 1) * C, 128 * l:128 * (l + 1)] = _dot(lhs, yf_s[c, :, 128 * l:128 * (l + 1)])
            pace.flush()

        def q_weights(p, odd, cols, n):
            w = q_s[p, 24 * odd:24 * odd + 24, cols]
            return jnp.concatenate([jnp.zeros((16, n), F32), w], 0) if odd else w

        def normalise(acc, odd):
            l = jnp.broadcast_to(acc[0:1] if odd else acc[23:24], (8, acc.shape[1]))
            inv_l = 1.0 / l
            return acc * jnp.concatenate([inv_l] * 3, 0), l

        def put_head(p, odd, cols, o):
            if odd:
                top = lax.broadcasted_iota(jnp.int32, (8, o.shape[1]), 0) < 4
                ot_s[p, 16:24, cols] = jnp.where(top, ot_s[p, 16:24, cols], o[0:8])
                ot_s[p, 24:40, cols] = o[8:24]
            else:
                ot_s[p, 0:24, cols] = o

        def pair_body(p, bad):
            head_cycles = (S // TQ) * (sum(nm) + 24 * NC)
            keep = keeps()
            pending = []
            accs = {}
            state = [bad]

            def pv(pace, odd, qb, t, probs):
                cols = slice(TQ * qb, TQ * (qb + 1))
                src = pb_s if odd else pa_s
                parts = [probs] if nm[t] else []
                if nm[t] < 128:
                    parts.append(src[vrow[t, nm[t]]:vrow[t, nm[t]] + 128 - nm[t], cols])
                lhs = _cat([pace.tie(vt_s[p, 24 * odd + r:24 * odd + r + 8, 128 * t:128 * (t + 1)], 8)
                            for r in (0, 8, 16)], 0)
                r = _dot(lhs, _cat(parts, 0))
                n, acc = accs.pop((odd, qb), (0, None))
                acc = r if acc is None else acc + r
                if n + 1 < NC:
                    accs[odd, qb] = (n + 1, acc)
                    return
                o, l = normalise(acc, odd)
                put_head(p, odd, cols, o)
                mag = jnp.abs(o[0:8]) + jnp.abs(o[8:16]) + jnp.abs(o[16:24])
                ok = (l >= L_LO) & (l <= L_HI) & (mag <= O_HI)
                for j in range(TQ // 128):
                    state[0] = jnp.where(ok[:, 128 * j:128 * (j + 1)], state[0], 1.0)

            for odd in range(2):
                nxt = jnp.minimum(p + 1, NPAIR - 1) if odd else p
                pace = _Pacer(score_jobs(nxt, 1 - odd, pa_s if odd else pb_s), head_cycles + (tail if odd else 0),
                              keep, 0 if odd else lead)
                for qb in range(S // TQ):
                    for t in range(NC):
                        if nm[t]:
                            kd = 24 + 16 * odd
                            lhs = _cat([pace.tie(kp_s[p, 128 * t + r:128 * t + r + 8, :], 8)
                                        for r in range(nm[t] - 8, -8, -8)], 0)
                            s = _dot(lhs[:, 0:kd], q_weights(p, odd, slice(TQ * qb, TQ * (qb + 1)), TQ))
                            s = _cat([s[r:r + 8] for r in range(nm[t] - 8, -8, -8)], 0)
                            if pending:
                                pv(pace, *pending.pop())
                            pending.append((odd, qb, t, jnp.exp2(s)))
                        else:
                            pv(pace, odd, qb, t, None)
                if odd:
                    pv(pace, *pending.pop())
                pace.flush()
            return state[0]

        with scope("attn"):
            bad = lax.fori_loop(0, NPAIR, pair_body, jnp.zeros((8, 128), F32))

        @pl.when(jnp.max(bad) > (-1.0 if force_slow else 0.0))
        def _():
            def slow_body(i, _):
                p = i // (S // 128)
                cols = pl.ds(pl.multiple_of((i % (S // 128)) * 128, 128), 128)
                for odd in range(2):
                    s = _dot(kp_s[p, :, 0:24 + 16 * odd], q_weights(p, odd, cols, 128))
                    e = jnp.exp2(s - jnp.max(s, axis=0, keepdims=True))
                    o, _ = normalise(_dot(vt_s[p, 24 * odd:24 * odd + 24, :], e), odd)
                    put_head(p, odd, cols, o)

            lax.fori_loop(0, NPAIR * (S // 128), slow_body, None)

        with scope("out"):
            cp_wo.wait()
            gw = g_v[...].astype(F32).reshape(1, D)
            dd = d_v[...].astype(F32).reshape(1, D)
            for i, (a, n) in enumerate(zip(oo, out_chunks)):
                a = int(a)
                o = jnp.concatenate([ot_s[p, :, a:a + n] for p in range(NPAIR)], 0).astype(BF16)
                att = _dot(o, wo_v[...], TN)
                xx = x_v[a:a + n, :].astype(F32)
                g = jax.nn.sigmoid(jnp.sum(xx * gw, axis=-1, keepdims=True))
                mix = xx * (y_s[a:a + n, :] + kv_s[a:a + n, :] * dd)
                out_v[a:a + n, :] = (g * att + (1.0 - g) * mix).astype(BF16)
                cp_o[i].start()
            for c in cp_o:
                c.wait()

    vm = pltpu.VMEM
    scratch = [
        vm((S, D), BF16), vm((D, D), BF16), vm((D, D), BF16), vm((D, D), BF16), vm((D, D), BF16),
        vm((S, D), BF16), vm((S, D), BF16), vm((4, D), BF16), vm((D, S), BF16), vm((D,), BF16), vm((D,), BF16),
        vm(_TABLES.shape, F32), vm((S, D), BF16),
        vm((D, D), U32), vm((NPAIR, S, 128), F32), vm((NPAIR, 48, S), F32), vm((NPAIR, 48, S), F32),
        vm((NPAIR, 40, S), F32), vm((max(nv, 8), S), F32), vm((max(nv, 8), S), F32), vm((S, D), F32),
        vm((NC, 2 * C, D), F32), vm((NC, 2 * C, D), F32), vm((NC, 2 * C, D), F32), vm((S, D), F32),
        pltpu.SemaphoreType.DMA((32,)),
    ]
    hbm = pl.BlockSpec(memory_space=pltpu.HBM)

    @jax.jit
    def run(A_x, A_wqkv, A_wo, B_q, B_k, B_v, B_shift_k, B_ssm_k, B_ssm_D, gate_w):
        out = pl.pallas_call(
            kernel,
            out_shape=jax.ShapeDtypeStruct((S, D), BF16),
            in_specs=[hbm] * 10,
            out_specs=hbm,
            scratch_shapes=scratch,
            compiler_params=pltpu.CompilerParams(vmem_limit_bytes=120 * 2 ** 20, flags=flags),
            name="gmix",
        )(A_x.reshape(S, D), A_wqkv, A_wo, B_k.reshape(S, D), B_v.reshape(S, D), B_shift_k.T, B_ssm_k,
          B_ssm_D, gate_w, _TABLES)
        return out.reshape(1, S, D)

    return run


pallas_gated_mix__mha_block__ssm_conv_h3__prompt_kernel = build()
```

```python
import functools

import jax
import jax.numpy as jnp
import numpy as np
from jax import lax
from jax.experimental import pallas as pl
from jax.experimental.pallas import tpu as pltpu

S, D, H = 2048, 640, 32
DH = D // H
NPAIR = H // 2
C = 128
NC = S // C
NL = D // 128
TQ = 512
NQB = S // TQ
F32, BF16, U32 = jnp.float32, jnp.bfloat16, jnp.uint32
QSCALE = float(DH ** -0.5 * np.log2(np.e))

L_LO, L_HI, O_HI, QK_HI = 2.0 ** -30, 2.0 ** 90, 2.0 ** 127, 2.0 ** 12

VPU_TILES, KEPT = 3, 32
BLOCKS = [(odd, k) for odd in range(2) for k in range(odd * KEPT // 32, 4 * VPU_TILES)]
STEPS = [(odd, t, qb) for odd in range(2) for qb in range(NQB) for t in range(VPU_TILES, NC)]
LATE = [(odd, t, qb) for odd in range(2) for t in range(VPU_TILES) for qb in range(NQB)] + STEPS[-1:]

K_STAGES = ((0, S, 0, 128), (0, 512, 128, 512), (512, S - 512, 128, 256), (512, S - 512, 384, 256))
KV_STAGES = ((0, 8), (8, 4), (12, 4), (16, 0))
EARLY = 4
FIRST_TABLES = (10, 14, 17, 20, len(BLOCKS) - 1)
TUNE = dict(lead=8, tail=0, col=2, free=6, frac=0.73, ahead=2, poff=2, kept_t=NC - 3, gap=56)

NN = (((1,), (0,)), ((), ()))
NT = (((1,), (1,)), ((), ()))
Q_LANES, V_LANES, T_LANES = slice(0, 128), slice(128, 256), slice(256, 384)


def _constants():
    w = 2.0 * np.pi * (np.arange(C)[:, None] + 0.25) / C
    t = np.arange(C)[None, :]
    mid = (C - 1) / 2
    inv = (w * (t[:, :C // 2] - mid)).T
    return np.concatenate([np.cos(w * t), -np.sin(w * t), np.cos(w * (t - mid)), -np.sin(w * (t - mid)),
                           np.cos(inv) / C, -np.sin(inv) / C, np.ones((48, C))], 0).astype(BF16)


_CONSTANTS = _constants()


def _dot(a, b, dims=NN):
    return lax.dot_general(a, b, dims, preferred_element_type=F32)


def _cat(xs, axis):
    return xs[0] if len(xs) == 1 else jnp.concatenate(xs, axis)


def _tile(i, n=128):
    return slice(n * i, n * (i + 1))


def _pack(v):
    return pltpu.bitcast(v.astype(BF16), U32)


def _side_by_side(v):
    return _cat([v[i] for i in range(v.shape[0])], 1)


def _reverse_groups(v):
    n = min(C, v.shape[0])
    return _cat([v[t + r:t + r + 8] for t in range(0, v.shape[0], n) for r in range(n - 8, -8, -8)], 0)


def _flip8(v):
    i = lax.broadcasted_iota(jnp.int32, v.shape, 0)
    v = pltpu.roll(v, 4, 0)
    v = jnp.where(i & 2 == 0, pltpu.roll(v, 6, 0), pltpu.roll(v, 2, 0))
    return jnp.where(i & 1 == 0, pltpu.roll(v, 7, 0), pltpu.roll(v, 1, 0))


def _halves(blk):
    return (_cat([blk[0:8], blk[16:24], blk[24:32]], 0),
            _cat([blk[8:16], pltpu.roll(blk[16:24], 6, 0), blk[32:40]], 0))


class _Pacer:
    def __init__(self, jobs, cycles=1, lead=0, col=0):
        self.jobs, self.cycles, self.lead, self.col = jobs, cycles, lead, col
        self.total = sum(w for w, _ in jobs)
        self.t = self.done = self.i = 0

    def after(self, res, dt=8):
        for r in range(0, res.shape[0], 8):
            self.t += dt
            self.mark = (res, r)
            while self.i < len(self.jobs) and self.done * self.cycles <= (self.t - self.lead) * self.total:
                self._run()

    def _run(self):
        w, job = self.jobs[self.i]
        res, r = self.mark
        job(res[r:r + 8, _tile(self.col)])
        self.done += w
        self.i += 1

    def flush(self):
        while self.i < len(self.jobs):
            self._run()


def _weave(jobs, extra, frac):
    out, k = [], 0
    for n, j in enumerate(jobs):
        out.append(j)
        while k < len(extra) and k * len(jobs) * frac <= n * len(extra):
            out.append(extra[k])
            k += 1
    return out + extra[k:]


def _kernel(x_hbm, wqkv_hbm, wo_hbm, k_hbm, v_hbm, sk_hbm, h_hbm, d_hbm, g_hbm, const_hbm, out_hbm,
            tables, x_v, wq_v, wk_v, wv_v, wo_v, k_v, v_v, h_v,
            wt_s, kr_s, ka_s, kb_s, qv_s, ot_s, p_s, kv_s, uf_s, hf_s, yf_s, gate_s,
            const_v, sk_v, d_v, g_v, sems):
    out_v = k_v

    def part(src, dst, idx):
        return src.at[idx], dst.at[idx]

    groups = [[part(x_hbm, x_v, (pl.ds(r, m), pl.ds(a, n)))] for r, m, a, n in K_STAGES]
    for i, (_, _, a, n) in enumerate(K_STAGES[:2]):
        groups[i].append((wqkv_hbm.at[pl.ds(a, n), pl.ds(D, D)], wk_v.at[pl.ds(a, n)]))
    groups[-1] += [(wqkv_hbm.at[:, pl.ds(0, D)], wq_v), (g_hbm, g_v), (sk_hbm, sk_v), (const_hbm, const_v)]
    for i, (a, n) in enumerate(KV_STAGES):
        groups.append([part(h_hbm, h_v, (slice(None), pl.ds(4 * i * C, 4 * C)))])
        if n:
            groups[-1] += [part(k_hbm, k_v, pl.ds(a * C, n * C)), part(v_hbm, v_v, pl.ds(a * C, n * C))]
    groups[-1].append((wqkv_hbm.at[:, pl.ds(2 * D, D)], wv_v))
    groups.append([(wo_hbm, wo_v), (d_hbm, d_v)])
    queue = [[pltpu.make_async_copy(a, b, sems.at[i + 1]) for a, b in g] for i, g in enumerate(groups)]

    def arrive():
        for c in queue.pop(0):
            c.wait()

    for group in queue:
        for c in group:
            c.start()
    p_s[...] = jnp.zeros(p_s.shape, U32)
    ot_s[0] = jnp.zeros(ot_s.shape[1:], F32)

    keep = [None]

    def load_keep():
        keep[0] = const_v[5 * C:5 * C + 16, :].astype(F32)[0:8] > 0.0

    def pin(v, mark):
        return v if mark is None else jnp.where(keep[0], v, mark)

    def fill_table(p, b, d, mark):
        odd, k = BLOCKS[b]
        r = 24 * odd + d if d < 8 else 8 + 4 * odd + d
        row = pin(jnp.broadcast_to(ka_s[p, r:r + 1, _tile(k)], (8, 128)), mark)
        tables[b][p if b == len(BLOCKS) - 1 else 0, d] = _cat([row] * 16, 0)[:, 0:112].T

    def project_t(w, xs, out, first, pace, held):
        top = lax.broadcasted_iota(jnp.int32, (8, 128), 0) < 4
        last = _dot(pltpu.bitcast(w(4)[:, 512:D], BF16), xs[:, 512:D], NT)
        pace.after(last)
        for n in range(4):
            r = _dot(pltpu.bitcast(w(n)[:, 0:512], BF16), xs[_tile(n), 0:512], NT)
            pace.after(r)
            r = r + last[:, _tile(n)]
            for j in range(r.shape[0] // 40):
                is_v, p = divmod(first + j, NPAIR)
                blk = r[_tile(j, 40)] if is_v else r[_tile(j, 40)] * QSCALE
                mid, fill = blk[16:24], float(is_v)
                out[p, n, 0:48, V_LANES if is_v else Q_LANES] = _cat(
                    [blk[0:16], jnp.where(top, mid, fill), jnp.where(top, fill, mid), blk[24:40]], 0)
                if not is_v and (p, n) not in held:
                    held[p, n] = (blk, out)
                elif not is_v:
                    prev, before = held.pop((p, n))
                    (b11, b21), (b12, b22) = _halves(prev), _halves(blk)
                    t1 = b12 - b11
                    t2 = b22 - t1
                    before[p, n, 0:48, T_LANES] = _cat([b21 - t2, t1], 0)
                    out[p, n, 0:48, T_LANES] = _cat([t2, b22 - b12], 0)

    def gate_job(r, mark):
        z = x_v[r:r + 16, :].astype(F32) * g_v[...].astype(F32).reshape(1, D)
        z = functools.reduce(jnp.add, [z[:, _tile(j)] for j in range(NL)])
        z = jnp.sum(_cat([pin(z[0:8], mark), pin(z[8:16], mark)], 0), axis=-1, keepdims=True)
        gate_s[r:r + 16, :] = jax.nn.sigmoid(jnp.broadcast_to(z, (16, 128)))

    halves = []
    for stage in K_STAGES:
        arrive()
        pace = _Pacer([])
        if stage == K_STAGES[-1]:
            load_keep()
            wqt = pltpu.bitcast(wq_v[...].T, U32)
            wt_s[0:D // 2 - DH * EARLY, :] = wqt[DH * EARLY:]
            jobs = [(14, functools.partial(gate_job, r)) for r in range(0, S, 16)]
            jobs += [(45, functools.partial(fill_table, 0, b, d)) for b in range(FIRST_TABLES[0]) for d in range(10)]
            pace = _Pacer(jobs, sum(w for w, _ in jobs), 300)
        for k, (lo, hi) in enumerate(halves):
            a11, a21, a12, a22 = lo[0:16], lo[16:32], hi[0:16], hi[16:32]
            s1 = a21 + a22
            s2 = s1 - a11
            factors = _cat([a11, a12, a12 - s2, a22, s1, s2, a11 - a21, a21], 0).T
            for p in range(NPAIR):
                ka_s[p, :, _tile(k)] = factors[40 * p:40 * p + 32]
        halves = []
        r0, m, a, n = stage
        for b in range(r0, r0 + m, 256):
            kk = _dot(x_v[b:b + 256, a:a + n], wk_v[a:a + n, :])
            for j in range(NL):
                pace.after(kk[:, _tile(j)], n / 64)
            if a:
                kk = kk + kv_s[b:b + 256, :]
            if a + n < D:
                kv_s[b:b + 256, :] = kk
                continue
            kr_s[b // 2:b // 2 + 128, :] = _pack(_reverse_groups(kk))
            for j in range(0, min(256, C * VPU_TILES - b), 32):
                feat = lax.rem(lax.broadcasted_iota(jnp.int32, (32, D), 1), 40)
                lo = _cat([kk[j + r:j + r + 8] for r in (0, 16, 8, 24)], 0)
                hi = jnp.where((feat >= 16) & (feat < 24), pltpu.roll(lo, D - 2, 1), pltpu.roll(lo, D - 8, 1))
                halves.append((lo, hi))
    held = {}
    for b in range(NQB):
        project_t(lambda _: wqt[0:DH * EARLY], x_v.at[_tile(b, TQ)], qv_s.at[:, _tile(b, 4)], 0, pace, held)
    pace.flush()

    def kv_job(st, c, l, r, mark):
        cols = _tile(l)
        if r == 0:
            w = [st["w"][j:j + 1, cols] for j in range(4)]
            cur = k_v[_tile(c), cols].astype(F32)
            prev = k_v[c * C - 16:c * C, cols].astype(F32)[8:] if c else jnp.zeros((8, 128), F32)
            k0 = _cat([prev, cur], 0)
            k1 = pltpu.roll(k0, 1, 0)
            far = pltpu.roll(k0 * w[2] + k1 * w[3], 2, 0)
            st["k"], st[c, l] = cur * w[0] + k1[8:] * w[1] + far[8:], []
        rows = slice(c * C + r, c * C + r + 16)
        v = v_v[rows, cols].astype(F32)
        kv = st["k"][r:r + 16] * _cat([pin(v[0:8], mark), pin(v[8:16], mark)], 0)
        kv_s[rows, cols] = kv
        st[c, l].append(kv)

    for i, (a, n) in enumerate(KV_STAGES):
        arrive()
        if i == len(KV_STAGES) - 1:
            wt_s[D // 2 - DH * EARLY:D - DH * EARLY, :] = pltpu.bitcast(wv_v[...].T, U32)
        load_keep()
        st = {"w": sk_v[...].astype(F32)}
        rounds = [(c, l) for c in range(a, a + n, 4) for l in range(NL)]
        pace = _Pacer([(1, functools.partial(kv_job, st, c + j, l, r))
                       for c, l in rounds for j in range(4) for r in range(0, C, 16)],
                      2 * C * (NL + len(rounds) - 2.5), 8)
        fills = _Pacer([(1, functools.partial(fill_table, 0, b, d))
                        for b in range(FIRST_TABLES[i], FIRST_TABLES[i + 1]) for d in range(10)],
                       2 * C * (NL + len(rounds) - 1.7))
        order = [((l - 1) / (NL - 1), 0, 4 * i, l) for l in range(NL)]
        order += [(m / (len(rounds) - 1), 1, c, l) for m, (c, l) in enumerate(rounds)]
        for _, is_kv, c, l in sorted(order):
            if is_kv:
                res = _dot(const_v[0:2 * C, :], _cat([_cat(st.pop((c + j, l)), 0) for j in range(4)], 1))
            else:
                res = _dot(const_v[2 * C:4 * C, :], _cat([h_v[_tile(l), _tile(c + j)] for j in range(4)], 0), NT)
            for j in range(4):
                for f in range(4):
                    (uf_s if is_kv else hf_s)[f % 2, c + j, f // 2, :, _tile(l)] = res[_tile(f, C // 2), _tile(j)]
            pace.after(res)
            fills.after(res)
        fills.flush()

    def spectral_job(st, its, at, which, a0, a1, mark):
        i = its[which]
        for a in range(a0, a1):
            hh = hf_s[(i, a, 0) + at]
            if which == 0:
                uu = uf_s[(i, a, 0) + at] + uf_s[(i, a, 1) + at]
            else:
                hi, uu = hf_s[(i, a, 1) + at], uf_s[(i, a, which - 1) + at]
                hh = hi - hh if which == 1 else hi + hh
            st["h", a], st["u", a] = hh, pin(uu, mark) if a == a0 else uu
            acc = [None, None]
            for b in range(a + 1):
                t = st["h", a - b] * st["u", b]
                acc[b % 2] = t if acc[b % 2] is None else acc[b % 2] + t
            yf_s[(its[0], a, which) + at] = acc[0] + acc[1] if a else acc[0]

    @pl.loop(0, 2)
    def _(i):
        load_keep()
        its = [i + ((i + w) >> 16) for w in range(3)]
        cuts, st = (0, 6, 9, 11, 13, 15, 16), {}
        jobs = [(sum(range(a0 + 1, a1 + 1)), functools.partial(spectral_job, st, its, (_tile(r, 8), _tile(l)), w, a0, a1))
                for r in range(C // 16) for l in range(NL) for w in range(3) for a0, a1 in zip(cuts, cuts[1:])]
        fills = [(0, functools.partial(fill_table, i * (NPAIR // 2) + p, len(BLOCKS) - 1, d))
                 for p in range(NPAIR // 2) for d in range(10)]
        rows, held = D - DH * EARLY, {}
        pace = _Pacer(_weave(jobs, fills, 0.6), 4 * rows * NL - 60, 8)
        for b in range(2):
            project_t(lambda n: wt_s.at[pl.ds(pl.multiple_of(32 * ((i + n + 5 * b) >> 16), 32), rows)],
                      x_v.at[pl.ds(pl.multiple_of((2 * i + b) * TQ, TQ), TQ)],
                      qv_s.at[:, pl.ds(4 * (2 * i + b), 4)], EARLY, pace, held)
        pace.flush()
        half = pl.ds(pl.multiple_of(i * (S // 4), S // 4), S // 4)
        for p in range(NPAIR):
            t, off = divmod(2 * DH * p, 128)
            blk = kr_s[half, _tile(t)]
            if off + 2 * DH > 128:
                blk = jnp.where(lax.broadcasted_iota(jnp.int32, blk.shape, 1) < 64, kr_s[half, _tile(t + 1)], blk)
            kb_s[p, half, :] = pltpu.roll(blk, 128 - off, 1) if off else blk

    arrive()

    def scores(p, odd, t, w, kept=0):
        if odd:
            w = _cat([jnp.zeros((16, w.shape[1]), F32), w], 0)
        keys = _cat(([kb_s[p, (C - kept) // 2:C // 2, :]] if kept else []) + [kb_s[p, _tile(t, C // 2), :]], 0)
        return _dot(pltpu.bitcast(keys, BF16)[:, 0:w.shape[0]], w)

    def late_rows(u, a=0, n=C):
        a += C * LATE.index(u)
        return slice(a // 2, (a + n) // 2)

    def late_pv(src, dst, u, probs):
        odd, t, qb = u
        r = _dot(qv_s[src, t, _tile(odd, 24), V_LANES], pltpu.bitcast(probs, BF16))
        ot_s[dst, _tile(odd, 24), _tile(qb, TQ)] += r
        return r

    @pl.loop(0, NPAIR)
    def _(p):
        load_keep()
        nxt, prv = jnp.minimum(p + 1, NPAIR - 1), jnp.maximum(p - 1, 0)
        old = {u: p_s[late_rows(u), :] for u in LATE}
        prod, bases = {}, {}

        def fresh(base, name, i):
            if (name, i) not in bases:
                bases[name, i] = base + ((p + i) >> 16)
            return bases[name, i]

        def score_job(b, qq, g, m, d0, pinned, mark):
            odd, k = BLOCKS[b]
            slot = fresh(p, "u", qq) if b == len(BLOCKS) - 1 else fresh(0, "t", qq)
            if d0 == 0:
                prod[m] = prod[5] + prod[4] if m == 2 else prod.get({1: 0, 5: 0, 6: 5, 3: 6}.get(m))
            for d in range(d0, d0 + 5):
                a = tables[b][slot, d, _tile(2 * m + g, 8), :]
                if pinned and d == d0 + TUNE["poff"]:
                    a = pin(a, mark)
                if m < 3:
                    r = 32 * odd + 8 * (m > 0) + d if d < 8 else 8 + 12 * odd + 2 * (m > 0) + d
                    lanes, qb = Q_LANES, 2 * qq + (m == 2)
                else:
                    r = 24 * ((m - 3) % 2) + (16 if d < 8 else 4) * odd + d
                    lanes, qb = T_LANES, 2 * qq + (m > 4)
                term = a * qv_s[fresh(p, "q", 2 * k + g), _tile(qb, 4), r:r + 1, lanes]
                prod[m] = term if prod[m] is None else prod[m] + term
            if d0 and m in (2, 3):
                s = [prod[2], prod[6] + prod[4]] if m == 2 else [prod[1], prod[3]]
                rows = late_rows((odd, k // 4, 2 * qq + (m == 2)), 32 * (k % 4) + 16 * g, 16)
                p_s[rows, :] = _pack(jnp.exp2(_cat([_side_by_side(v) for v in s], 0)))

        jobs, due = [], {}
        for b, (odd, k) in enumerate(BLOCKS):
            for qb in range(NQB):
                due.setdefault((odd, k // 4, qb), sum(w for w, _ in jobs) + 38 - TUNE["gap"] * (3 - qb))
            work = [(qq, g, m, d0) for qq in range(2) for g in range(2) for m in (0, 1, 5, 6, 3, 4, 2) for d0 in (0, 5)]
            pinned = [b > 0 or n >= TUNE["free"] for n in range(len(work))]
            fills = [(0, functools.partial(fill_table, nxt, b - 1, d)) for d in range(10 if b else 0)]
            jobs += _weave([(int(f), functools.partial(score_job, b, *w, f)) for w, f in zip(work, pinned)],
                           fills, TUNE["frac"] if b == len(BLOCKS) - 1 else 1.0)
        cycles = C * len(STEPS) + 24 * 2 * NQB * NC + NQB * KEPT
        pace = _Pacer(jobs, cycles - TUNE["lead"] + TUNE["tail"], TUNE["lead"], TUNE["col"])
        due[LATE[-1]] = pace.total - 56
        todo, acc, probs = sorted(LATE, key=due.get), None, None
        for n, (odd, t, qb) in enumerate(STEPS):
            kept = KEPT if odd and t == TUNE["kept_t"] else 0
            w = _side_by_side(qv_s[fresh(p, "w", t), _tile(qb, 4), _tile(odd, 24), Q_LANES])
            s = scores(fresh(p, "k", odd * NQB + qb), odd, t, w, kept)
            pace.after(s)
            if kept:
                p_s[late_rows((odd, 0, qb), 0, kept), :] = _pack(jnp.exp2(_reverse_groups(s[0:kept])))
            if n:
                o, u, c = STEPS[n - 1]
                r = _dot(qv_s[fresh(p, "p", c), u, _tile(o, 24), V_LANES], probs)
                pace.after(r)
                acc = r if acc is None else acc + r
                if u == NC - 1 or n == len(STEPS) - 1:
                    ot_s[p + 1, _tile(o, 24), _tile(c, TQ)], acc = acc, None
            if todo and (n + TUNE["ahead"]) * pace.total >= due[todo[0]] * len(STEPS):
                u = todo.pop(0)
                pace.after(late_pv(fresh(prv, "v", u[2]), fresh(p, "o", len(todo)), u, old[u]))
            probs = jnp.exp2(_reverse_groups(s[kept:]))
        pace.flush()
        assert not todo
        p_s[late_rows(LATE[-1]), :] = _pack(probs)

    for u in sorted(LATE, key=lambda u: u[2]):
        late_pv(NPAIR - 1, NPAIR, u, p_s[late_rows(u), :])

    def normalise(p, cols, mark=None):
        top = lax.broadcasted_iota(jnp.int32, (8, 128), 0) < 4
        acc = ot_s[p + 1, :, cols]
        l = pin(jnp.where(top, acc[24:32], acc[16:24]), mark)
        inv = 1.0 / l
        even, odd = acc[0:24] * inv[7:8], acc[24:48] * inv[0:1]
        blk = [even[0:8], even[8:16], jnp.where(top, even[16:24], odd[0:8]), odd[8:16], odd[16:24]]
        size = functools.reduce(jnp.add, [jnp.abs(b) for b in blk])
        return _cat(blk, 0), (l >= L_LO) & (l <= L_HI) & (size <= O_HI)

    def long_conv(c, cols):
        def spectrum(c):
            k = [_cat([yf_s[j, c, w, :, cols] for j in range(2)], 0) for w in range(3)]
            return k[0] - k[2], k[0] + k[1]

        (re0, im0), (re1, im1) = spectrum(c), spectrum(c + 1)
        re1, im1 = re1 - im0, im1 + re0
        if not isinstance(c, int):
            re, im = spectrum(jnp.maximum(c - 1, 0))
            re0, im0 = re0 - jnp.where(c > 0, im, 0.0), im0 + jnp.where(c > 0, re, 0.0)
        elif c:
            re, im = spectrum(c - 1)
            re0, im0 = re0 - im, im0 + re
        even = _dot(const_v[4 * C:4 * C + C // 2, :], _cat([re0, re1], 1))
        odd = _dot(const_v[4 * C + C // 2:5 * C, :], _cat([im0, im1], 1))
        back = even - odd
        y = _cat([even + odd] + [_flip8(back[r:r + 8]) for r in range(C // 2 - 8, -8, -8)], 0)
        return _cat([y[:, 0:128], y[:, 128:256]], 0)

    def mix(c, rows, o, pace, done):
        o = o.astype(BF16).T
        corner = _cat([_dot(o[_tile(r, 64), 512:D], wo_v[512:D, 512:D]) for r in range(4)], 0)
        edge = _cat([_dot(o[:, 512:D], wo_v[512:D, 0:512]), corner], 1)
        pace.after(edge)
        skip = d_v[...].astype(F32).reshape(1, D)
        for l in range(NL):
            cols = _tile(l)
            y = long_conv(c, cols)
            att = _dot(o[:, 0:512], wo_v[0:512, cols])
            pace.after(att)
            b = (y + kv_s[rows, cols] * skip[:, cols]) * x_v[rows, cols].astype(F32)
            g = gate_s[rows, :]
            out_v[rows, cols] = (g * (att + edge[:, cols]) + (1.0 - g) * b).astype(BF16)
            done(l)
        pace.flush()

    load_keep()
    st = {name: jnp.zeros((8, 128), F32) for name in ("bad", "q", "k")}
    sent = []

    def norm_job(p, c, mark):
        st[p, c], ok = normalise(p, _tile(c), mark)
        st["bad"] = jnp.where(ok, st["bad"], 1.0)
        seen = [("q", qv_s[p, c, 0:48, Q_LANES])] + ([("k", ka_s[p, :, _tile(c)])] if c < 4 * VPU_TILES else [])
        for name, v in seen:
            v = functools.reduce(jnp.maximum, [jnp.abs(v[r:r + 8]) for r in range(0, v.shape[0], 8)])
            st[name] = jnp.maximum(st[name], pin(v, mark))

    def send(c, l):
        if c + 2 < NC:
            cols = {NL - 1: slice(None)}.get(l)
        else:
            cols = {NL - 2: pl.ds(0, D - 128), NL - 1: pl.ds(D - 128, 128)}.get(l)
        if cols is not None:
            sent.append(pltpu.make_async_copy(*part(out_v, out_hbm, (pl.ds(c * C, 2 * C), cols)), sems.at[0]))
            sent[-1].start()

    for p in range(NPAIR):
        for c in range(2):
            norm_job(p, c, None)
    for c in range(0, NC, 2):
        o = _cat([_cat([st.pop((p, j)) for p in range(NPAIR)], 0) for j in (c, c + 1)], 1)
        jobs = [(1, functools.partial(norm_job, p, j)) for p in range(NPAIR) for j in (c + 2, c + 3) if j < NC]
        mix(c, _tile(c // 2, 2 * C), o, _Pacer(jobs, 8 * C), functools.partial(send, c))
    redo = (jnp.max(st["bad"]) > 0.0) | (jnp.max(st["q"]) * jnp.max(st["k"]) > QK_HI)
    for c in sent:
        c.wait()

    @pl.when(redo)
    def _():
        @pl.loop(0, NPAIR * NC)
        def _(i):
            p, c = i // NC, i % NC
            for odd in range(2):
                w = qv_s[p, c, _tile(odd, 24), Q_LANES]
                s = _reverse_groups(_cat([scores(p, odd, t, w) for t in range(NC)], 0))
                e = jnp.exp2(s - jnp.max(s, axis=0, keepdims=True)) * (1.0 / S)
                ot_s[p + 1, _tile(odd, 24), pl.ds(pl.multiple_of(c * C, C), C)] = _dot(
                    _side_by_side(qv_s[p, :, _tile(odd, 24), V_LANES]), e)

        @pl.loop(0, NC // 2)
        def _(i):
            both = [pl.ds(pl.multiple_of((2 * i + j) * C, C), C) for j in range(2)]
            o = _cat([_cat([normalise(p, cols)[0] for p in range(NPAIR)], 0) for cols in both], 1)
            mix(2 * i, pl.ds(pl.multiple_of(2 * i * C, 2 * C), 2 * C), o, _Pacer([]), lambda l: None)

        everything = pltpu.make_async_copy(out_v, out_hbm, sems.at[0])
        everything.start()
        everything.wait()


@jax.jit
def pallas_gated_mix__mha_block__ssm_conv_h3__prompt_kernel(
    A_x: jax.Array,
    A_wqkv: jax.Array,
    A_wo: jax.Array,
    B_q: jax.Array,
    B_k: jax.Array,
    B_v: jax.Array,
    B_shift_k: jax.Array,
    B_ssm_k: jax.Array,
    B_ssm_D: jax.Array,
    gate_w: jax.Array,
):
    del B_q
    vm = pltpu.VMEM
    scratch = [
        [vm((NPAIR if b == len(BLOCKS) - 1 else 1, 10, 112, 128), F32) for b in range(len(BLOCKS))],
        vm((S, D), BF16), vm((D, D), BF16), vm((D, D), BF16), vm((D, D), BF16), vm((D, D), BF16),
        vm((S, D), BF16), vm((S, D), BF16), vm((D, S), BF16),
        vm((D, D), U32), vm((S // 2, D), U32), vm((NPAIR, 32, 4 * C * VPU_TILES), F32),
        vm((NPAIR, S // 2, 128), U32), vm((NPAIR, NC, 56, 384), F32), vm((NPAIR + 1, 48, S), F32),
        vm((C // 2 * len(LATE), TQ), U32), vm((S, D), F32),
        vm((2, NC, 2, C // 2, D), F32), vm((2, NC, 2, C // 2, D), F32), vm((2, NC, 3, C // 2, D), F32),
        vm((S, 128), F32),
        vm(_CONSTANTS.shape, BF16), vm((4, D), BF16), vm((D,), BF16), vm((D,), BF16),
        pltpu.SemaphoreType.DMA((len(K_STAGES) + len(KV_STAGES) + 2,)),
    ]
    hbm = pl.BlockSpec(memory_space=pltpu.HBM)
    out = pl.pallas_call(
        _kernel,
        out_shape=jax.ShapeDtypeStruct((S, D), BF16),
        in_specs=[hbm] * 10,
        out_specs=hbm,
        scratch_shapes=scratch,
        compiler_params=pltpu.CompilerParams(vmem_limit_bytes=127 * 2 ** 20),
        name="gmix",
    )(A_x.reshape(S, D), A_wqkv, A_wo, B_k.reshape(S, D), B_v.reshape(S, D), B_shift_k.T, B_ssm_k,
      B_ssm_D, gate_w, _CONSTANTS)
    return out.reshape(1, S, D)
```

```python
import functools

import jax
import jax.numpy as jnp
import numpy as np
from jax import lax
from jax.experimental import pallas as pl
from jax.experimental.pallas import tpu as pltpu

S, D, H = 2048, 640, 32
DH = D // H
NPAIR = H // 2
C = 128
NC = S // C
NL = D // 128
TQ = 512
NQB = S // TQ
F32, BF16, U32 = jnp.float32, jnp.bfloat16, jnp.uint32
QSCALE = float(DH ** -0.5 * np.log2(np.e))

L_LO, L_HI, O_HI, QK_HI = 2.0 ** -30, 2.0 ** 90, 2.0 ** 127, 2.0 ** 12

VPU_TILES, KEPT = 3, 32
BLOCKS = [(odd, k) for odd in range(2) for k in range(odd * KEPT // 32, 4 * VPU_TILES)]
STEPS = [(odd, t, qb) for odd in range(2) for qb in range(NQB) for t in range(VPU_TILES, NC)]
LATE = [(odd, t, qb) for odd in range(2) for t in range(VPU_TILES) for qb in range(NQB)] + STEPS[-1:]

K_STAGES = ((0, S, 0, 128), (0, 512, 128, 512), (512, S - 512, 128, 256), (512, S - 512, 384, 256))
KV_STAGES = ((0, 8), (8, 4), (12, 4), (16, 0))
EARLY = 4
FIRST_TABLES = (8, 13, 17, 21, len(BLOCKS) - 1)

NN = (((1,), (0,)), ((), ()))
NT = (((1,), (1,)), ((), ()))
Q_LANES, V_LANES, T_LANES = slice(0, 128), slice(128, 256), slice(256, 384)


def _constants():
    w = 2.0 * np.pi * (np.arange(C)[:, None] + 0.25) / C
    t = np.arange(C)[None, :]
    mid = (C - 1) / 2
    inv = (w * (t[:, :C // 2] - mid)).T
    return np.concatenate([np.cos(w * t), -np.sin(w * t), np.cos(w * (t - mid)), -np.sin(w * (t - mid)),
                           np.cos(inv) / C, -np.sin(inv) / C, np.ones((48, C))], 0).astype(BF16)


_CONSTANTS = _constants()


def _dot(a, b, dims=NN):
    return lax.dot_general(a, b, dims, preferred_element_type=F32)


def _cat(xs, axis):
    return xs[0] if len(xs) == 1 else jnp.concatenate(xs, axis)


def _tile(i, n=128):
    return slice(n * i, n * (i + 1))


def _pack(v):
    return pltpu.bitcast(v.astype(BF16), U32)


def _peak(v):
    return functools.reduce(jnp.maximum, [jnp.abs(v[r:r + 8]) for r in range(0, v.shape[0], 8)])


def _side_by_side(v):
    return _cat([v[i] for i in range(v.shape[0])], 1)


def _reverse_groups(v):
    n = min(C, v.shape[0])
    return _cat([v[t + r:t + r + 8] for t in range(0, v.shape[0], n) for r in range(n - 8, -8, -8)], 0)


def _flip8(v):
    i = lax.broadcasted_iota(jnp.int32, v.shape, 0)
    v = pltpu.roll(v, 4, 0)
    v = jnp.where(i & 2 == 0, pltpu.roll(v, 6, 0), pltpu.roll(v, 2, 0))
    return jnp.where(i & 1 == 0, pltpu.roll(v, 7, 0), pltpu.roll(v, 1, 0))


def _halves(blk):
    return (_cat([blk[0:8], blk[16:24], blk[24:32]], 0),
            _cat([blk[8:16], pltpu.roll(blk[16:24], 6, 0), blk[32:40]], 0))


class _Pacer:
    def __init__(self, jobs, cycles=1, lead=0, col=0):
        self.jobs, self.cycles, self.lead, self.col = jobs, cycles, lead, col
        self.total = sum(w for w, _ in jobs)
        self.t = self.done = self.i = 0

    def after(self, res, dt=8):
        for r in range(0, res.shape[0], 8):
            self.t += dt
            self.mark = (res, r)
            while self.i < len(self.jobs) and self.done * self.cycles <= (self.t - self.lead) * self.total:
                self._run()

    def _run(self):
        w, job = self.jobs[self.i]
        res, r = self.mark
        job(res[r:r + 8, _tile(self.col)])
        self.done += w
        self.i += 1

    def flush(self):
        while self.i < len(self.jobs):
            self._run()


def _weave(jobs, extra, frac):
    out, k = [], 0
    for n, j in enumerate(jobs):
        out.append(j)
        while k < len(extra) and k * len(jobs) * frac <= n * len(extra):
            out.append(extra[k])
            k += 1
    return out + extra[k:]


def _kernel(x_hbm, wqkv_hbm, wo_hbm, k_hbm, v_hbm, sk_hbm, h_hbm, d_hbm, g_hbm, const_hbm, out_hbm,
            tables, x_v, wq_v, wk_v, wv_v, wo_v, k_v, v_v, h_v,
            wt_s, kr_s, ka_s, kb_s, qv_s, ot_s, p_s, uf_s, hf_s, yf_s, gate_s,
            const_v, sk_v, d_v, g_v, sems):
    kv_v, out_v = v_v, k_v

    def part(src, dst, idx):
        return src.at[idx], dst.at[idx]

    groups = [[part(x_hbm, x_v, (pl.ds(r, m), pl.ds(a, n)))] for r, m, a, n in K_STAGES]
    for i, (_, _, a, n) in enumerate(K_STAGES[:2]):
        groups[i].append((wqkv_hbm.at[pl.ds(a, n), pl.ds(D, D)], wk_v.at[pl.ds(a, n)]))
    groups[-1] += [(wqkv_hbm.at[:, pl.ds(0, D)], wq_v), (g_hbm, g_v), (sk_hbm, sk_v), (const_hbm, const_v)]
    for i, (a, n) in enumerate(KV_STAGES):
        groups.append([part(h_hbm, h_v, (slice(None), pl.ds(4 * i * C, 4 * C)))])
        if n:
            groups[-1] += [part(k_hbm, k_v, pl.ds(a * C, n * C)), part(v_hbm, v_v, pl.ds(a * C, n * C))]
    groups[-1].append((wqkv_hbm.at[:, pl.ds(2 * D, D)], wv_v))
    groups.append([(wo_hbm, wo_v), (d_hbm, d_v)])
    queue = [[pltpu.make_async_copy(a, b, sems.at[i + 1]) for a, b in g] for i, g in enumerate(groups)]

    def arrive():
        for c in queue.pop(0):
            c.wait()

    for group in queue:
        for c in group:
            c.start()
    p_s[...] = jnp.zeros(p_s.shape, U32)
    ot_s[0] = jnp.zeros(ot_s.shape[1:], F32)

    keep = [None]

    def load_keep():
        keep[0] = const_v[5 * C:5 * C + 16, :].astype(F32)[0:8] > 0.0

    def pin(v, mark):
        return v if mark is None else jnp.where(keep[0], v, mark)

    def fill_table(p, b, d, mark):
        odd, k = BLOCKS[b]
        r = 24 * odd + d if d < 8 else 8 + 4 * odd + d
        row = pin(jnp.broadcast_to(ka_s[p, r:r + 1, _tile(k)], (8, 128)), mark)
        tables[b][p if b == len(BLOCKS) - 1 else 0, d] = _cat([row] * 16, 0)[:, 0:112].T

    def project_t(w, xs, out, first, pace, held):
        top = lax.broadcasted_iota(jnp.int32, (8, 128), 0) < 4
        last = _dot(pltpu.bitcast(w(4)[:, 512:D], BF16), xs[:, 512:D], NT)
        pace.after(last)
        for n in range(4):
            r = _dot(pltpu.bitcast(w(n)[:, 0:512], BF16), xs[_tile(n), 0:512], NT)
            pace.after(r)
            r = r + last[:, _tile(n)]
            for j in range(r.shape[0] // 40):
                is_v, p = divmod(first + j, NPAIR)
                blk = r[_tile(j, 40)] if is_v else r[_tile(j, 40)] * QSCALE
                mid, fill = blk[16:24], float(is_v)
                out[p, n, 0:48, V_LANES if is_v else Q_LANES] = _cat(
                    [blk[0:16], jnp.where(top, mid, fill), jnp.where(top, fill, mid), blk[24:40]], 0)
                if not is_v and (p, n) not in held:
                    held[p, n] = (blk, out)
                elif not is_v:
                    prev, before = held.pop((p, n))
                    (b11, b21), (b12, b22) = _halves(prev), _halves(blk)
                    t1 = b12 - b11
                    t2 = b22 - t1
                    before[p, n, 0:48, T_LANES] = _cat([b21 - t2, t1], 0)
                    out[p, n, 0:48, T_LANES] = _cat([t2, b22 - b12], 0)

    def gate_job(r, mark):
        z = x_v[r:r + 16, :].astype(F32) * g_v[...].astype(F32).reshape(1, D)
        z = functools.reduce(jnp.add, [z[:, _tile(j)] for j in range(NL)])
        z = jnp.sum(_cat([pin(z[0:8], mark), pin(z[8:16], mark)], 0), axis=-1, keepdims=True)
        gate_s[r:r + 16, :] = jax.nn.sigmoid(jnp.broadcast_to(z, (16, 128)))

    halves, partial, k_peak = [], {}, 0.0
    for stage in K_STAGES:
        arrive()
        pace = _Pacer([])
        if stage == K_STAGES[-1]:
            load_keep()
            wqt = pltpu.bitcast(wq_v[...].T, U32)
            wt_s[0:D // 2 - DH * EARLY, :] = wqt[DH * EARLY:]
            jobs = [(23, functools.partial(gate_job, r)) for r in range(0, S, 16)]
            jobs += [(45, functools.partial(fill_table, 0, b, d)) for b in range(FIRST_TABLES[0]) for d in range(10)]
            pace = _Pacer(jobs, sum(w for w, _ in jobs), 150)
        for k, (lo, hi) in enumerate(halves):
            a11, a21, a12, a22 = lo[0:16], lo[16:32], hi[0:16], hi[16:32]
            s1 = a21 + a22
            s2 = s1 - a11
            factors = _cat([a11, a12, a12 - s2, a22, s1, s2, a11 - a21, a21], 0).T
            k_peak = jnp.maximum(k_peak, _peak(factors))
            for p in range(NPAIR):
                ka_s[p, :, _tile(k)] = factors[40 * p:40 * p + 32]
        halves = []
        r0, m, a, n = stage
        for b in range(r0, r0 + m, 256):
            kk = _dot(x_v[b:b + 256, a:a + n], wk_v[a:a + n, :])
            for j in range(NL):
                pace.after(kk[:, _tile(j)], n / 64)
            if a:
                kk = kk + partial[b]
            if a + n < D:
                partial[b] = kk
                continue
            kr_s[b // 2:b // 2 + 128, :] = _pack(_reverse_groups(kk))
            for j in range(0, min(256, C * VPU_TILES - b), 32):
                feat = lax.rem(lax.broadcasted_iota(jnp.int32, (32, D), 1), 40)
                lo = _cat([kk[j + r:j + r + 8] for r in (0, 16, 8, 24)], 0)
                hi = jnp.where((feat >= 16) & (feat < 24), pltpu.roll(lo, D - 2, 1), pltpu.roll(lo, D - 8, 1))
                halves.append((lo, hi))
    held = {}
    for b in range(NQB):
        project_t(lambda _: wqt[0:DH * EARLY], x_v.at[_tile(b, TQ)], qv_s.at[:, _tile(b, 4)], 0, pace, held)
    pace.flush()

    def kv_job(st, c, l, r, mark):
        cols = _tile(l)
        if r == 0:
            w = [st["w"][j:j + 1, cols] for j in range(4)]
            cur = k_v[_tile(c), cols].astype(F32)
            prev = k_v[c * C - 16:c * C, cols].astype(F32)[8:] if c else jnp.zeros((8, 128), F32)
            k0 = _cat([prev, cur], 0)
            k1 = pltpu.roll(k0, 1, 0)
            far = pltpu.roll(k0 * w[2] + k1 * w[3], 2, 0)
            st["k"], st[c, l] = cur * w[0] + k1[8:] * w[1] + far[8:], []
        rows = slice(c * C + r, c * C + r + 16)
        v = v_v[rows, cols].astype(F32)
        kv = st["k"][r:r + 16] * _cat([pin(v[0:8], mark), pin(v[8:16], mark)], 0)
        kv_v[rows, cols] = kv.astype(BF16)
        st[c, l].append(kv)

    for i, (a, n) in enumerate(KV_STAGES):
        arrive()
        if i == len(KV_STAGES) - 1:
            wt_s[D // 2 - DH * EARLY:D - DH * EARLY, :] = pltpu.bitcast(wv_v[...].T, U32)
        load_keep()
        st = {"w": sk_v[...].astype(F32)}
        rounds = [(c, l) for c in range(a, a + n, 4) for l in range(NL)]
        pace = _Pacer([(1, functools.partial(kv_job, st, c + j, l, r))
                       for c, l in rounds for j in range(4) for r in range(0, C, 16)],
                      2 * C * (NL + len(rounds) - 2.5), 8)
        fills = _Pacer([(1, functools.partial(fill_table, 0, b, d))
                        for b in range(FIRST_TABLES[i], FIRST_TABLES[i + 1]) for d in range(10)],
                       2 * C * (NL + len(rounds) - 1.5))
        order = [((l - 1) / (NL - 1), 0, 4 * i, l) for l in range(NL)]
        order += [(m / (len(rounds) - 1), 1, c, l) for m, (c, l) in enumerate(rounds)]
        for _, is_kv, c, l in sorted(order):
            if is_kv:
                res = _dot(const_v[0:2 * C, :], _cat([_cat(st.pop((c + j, l)), 0) for j in range(4)], 1))
            else:
                res = _dot(const_v[2 * C:4 * C, :], _cat([h_v[_tile(l), _tile(c + j)] for j in range(4)], 0), NT)
            for j in range(4):
                for f in range(4):
                    (uf_s if is_kv else hf_s)[f % 2, c + j, f // 2, :, _tile(l)] = res[_tile(f, C // 2), _tile(j)]
            pace.after(res)
            fills.after(res)
        fills.flush()

    def spectral_job(st, its, at, which, a0, a1, mark):
        i = its[which]
        for a in range(a0, a1):
            hh = hf_s[(i, a, 0) + at]
            if which == 0:
                uu = uf_s[(i, a, 0) + at] + uf_s[(i, a, 1) + at]
            else:
                hi, uu = hf_s[(i, a, 1) + at], uf_s[(i, a, which - 1) + at]
                hh = hi - hh if which == 1 else hi + hh
            st["h", a], st["u", a] = hh, pin(uu, mark) if a == a0 else uu
            acc = [None, None]
            for b in range(a + 1):
                t = st["h", a - b] * st["u", b]
                acc[b % 2] = t if acc[b % 2] is None else acc[b % 2] + t
            yf_s[(its[0], a, which) + at] = acc[0] + acc[1] if a else acc[0]

    @pl.loop(0, 2)
    def _(i):
        load_keep()
        its = [i + ((i + w) >> 16) for w in range(3)]
        cuts, st = (0, 6, 9, 11, 13, 15, 16), {}
        jobs = [(sum(range(a0 + 1, a1 + 1)), functools.partial(spectral_job, st, its, (_tile(r, 8), _tile(l)), w, a0, a1))
                for r in range(C // 16) for l in range(NL) for w in range(3) for a0, a1 in zip(cuts, cuts[1:])]
        fills = [(0, functools.partial(fill_table, i * (NPAIR // 2) + p, len(BLOCKS) - 1, d))
                 for p in range(NPAIR // 2) for d in range(10)]
        rows, held = D - DH * EARLY, {}
        pace = _Pacer(_weave(jobs, fills, 0.6), 4 * rows * NL - 60, 8)
        for b in range(2):
            project_t(lambda n: wt_s.at[pl.ds(pl.multiple_of(32 * ((i + n + 5 * b) >> 16), 32), rows)],
                      x_v.at[pl.ds(pl.multiple_of((2 * i + b) * TQ, TQ), TQ)],
                      qv_s.at[:, pl.ds(4 * (2 * i + b), 4)], EARLY, pace, held)
        pace.flush()
        half = pl.ds(pl.multiple_of(i * (S // 4), S // 4), S // 4)
        for p in range(NPAIR):
            t, off = divmod(2 * DH * p, 128)
            blk = kr_s[half, _tile(t)]
            if off + 2 * DH > 128:
                blk = jnp.where(lax.broadcasted_iota(jnp.int32, blk.shape, 1) < 64, kr_s[half, _tile(t + 1)], blk)
            kb_s[p, half, :] = pltpu.roll(blk, 128 - off, 1) if off else blk

    arrive()

    def scores(p, odd, t, w, kept=0):
        if odd:
            w = _cat([jnp.zeros((16, w.shape[1]), F32), w], 0)
        keys = _cat(([kb_s[p, (C - kept) // 2:C // 2, :]] if kept else []) + [kb_s[p, _tile(t, C // 2), :]], 0)
        return _dot(pltpu.bitcast(keys, BF16)[:, 0:w.shape[0]], w)

    def late_rows(u, a=0, n=C):
        a += C * LATE.index(u)
        return slice(a // 2, (a + n) // 2)

    def late_pv(src, dst, u, probs):
        odd, t, qb = u
        r = _dot(qv_s[src, t, _tile(odd, 24), V_LANES], pltpu.bitcast(probs, BF16))
        ot_s[dst, _tile(odd, 24), _tile(qb, TQ)] += r
        return r

    @pl.loop(0, NPAIR)
    def _(p):
        load_keep()
        nxt, prv = jnp.minimum(p + 1, NPAIR - 1), jnp.maximum(p - 1, 0)
        old = {u: p_s[late_rows(u), :] for u in LATE}
        prod, bases = {}, {}

        def fresh(base, name, i):
            if (name, i) not in bases:
                bases[name, i] = base + ((p + i) >> 16)
            return bases[name, i]

        def score_job(b, steps, pinned, mark):
            odd, k = BLOCKS[b]
            for n, (qq, g, m, d) in enumerate(steps):
                if d == 0:
                    prod[m] = prod[5] + prod[4] if m == 2 else prod.get({1: 0, 5: 0, 6: 5, 3: 6}.get(m))
                slot = fresh(p, "u", qq) if b == len(BLOCKS) - 1 else fresh(0, "t", qq)
                a = tables[b][slot, d, _tile(2 * m + g, 8), :]
                if pinned and n == 2:
                    a = pin(a, mark)
                if m < 3:
                    r = 32 * odd + 8 * (m > 0) + d if d < 8 else 8 + 12 * odd + 2 * (m > 0) + d
                    lanes, qb = Q_LANES, 2 * qq + (m == 2)
                else:
                    r = 24 * ((m - 3) % 2) + (16 if d < 8 else 4) * odd + d
                    lanes, qb = T_LANES, 2 * qq + (m > 4)
                term = a * qv_s[fresh(p, "q", 2 * k + g), _tile(qb, 4), r:r + 1, lanes]
                prod[m] = term if prod[m] is None else prod[m] + term
                if d == 9 and m in (2, 3):
                    s = [prod[2], prod[6] + prod[4]] if m == 2 else [prod[1], prod[3]]
                    rows = late_rows((odd, k // 4, 2 * qq + (m == 2)), 32 * (k % 4) + 16 * g, 16)
                    p_s[rows, :] = _pack(jnp.exp2(_cat([_side_by_side(v) for v in s], 0)))

        jobs, due = [], {}
        for b, (odd, k) in enumerate(BLOCKS):
            for qb in range(NQB):
                due.setdefault((odd, k // 4, qb), sum(w for w, _ in jobs) + 38 - 56 * (3 - qb))
            work = [(qq, g, m, d) for qq in range(2) for g in range(2) for m in (0, 1, 5, 6, 3, 4, 2) for d in range(10)]
            work = [work[n:n + 5] for n in range(0, len(work), 5)]
            pinned = [b > 0 or n >= 6 for n in range(len(work))]
            fills = [(0, functools.partial(fill_table, nxt, b - 1, d)) for d in range(10 if b else 0)]
            jobs += _weave([(int(f), functools.partial(score_job, b, w, f)) for w, f in zip(work, pinned)],
                           fills, 0.73 if b == len(BLOCKS) - 1 else 1.0)
        cycles = C * len(STEPS) + 24 * 2 * NQB * NC + NQB * KEPT
        pace = _Pacer(jobs, cycles - 8, lead=8, col=2)
        due[LATE[-1]] = pace.total - 56
        todo, acc, probs = sorted(LATE, key=due.get), None, None
        for n, (odd, t, qb) in enumerate(STEPS):
            kept = KEPT if odd and t == NC - 2 else 0
            w = _side_by_side(qv_s[fresh(p, "w", t), _tile(qb, 4), _tile(odd, 24), Q_LANES])
            s = scores(fresh(p, "k", odd * NQB + qb), odd, t, w, kept)
            pace.after(s)
            if kept:
                p_s[late_rows((odd, 0, qb), 0, kept), :] = _pack(jnp.exp2(_reverse_groups(s[0:kept])))
            if n:
                o, u, c = STEPS[n - 1]
                r = _dot(qv_s[fresh(p, "p", c), u, _tile(o, 24), V_LANES], probs)
                pace.after(r)
                acc = r if acc is None else acc + r
                if u == NC - 1 or n == len(STEPS) - 1:
                    ot_s[p + 1, _tile(o, 24), _tile(c, TQ)], acc = acc, None
            if todo and (n + 3) * pace.total >= due[todo[0]] * len(STEPS):
                u = todo.pop(0)
                pace.after(late_pv(fresh(prv, "v", u[2]), fresh(p, "o", len(todo)), u, old[u]))
            probs = jnp.exp2(_reverse_groups(s[kept:]))
        pace.flush()
        assert not todo
        p_s[late_rows(LATE[-1]), :] = _pack(probs)

    for u in sorted(LATE, key=lambda u: u[2]):
        late_pv(NPAIR - 1, NPAIR, u, p_s[late_rows(u), :])

    def normalise(p, cols, mark=None):
        top = lax.broadcasted_iota(jnp.int32, (8, 128), 0) < 4
        acc = ot_s[p + 1, :, cols]
        l = pin(jnp.where(top, acc[24:32], acc[16:24]), mark)
        inv = 1.0 / l
        even, odd = acc[0:24] * inv[7:8], acc[24:48] * inv[0:1]
        blk = [even[0:8], even[8:16], jnp.where(top, even[16:24], odd[0:8]), odd[8:16], odd[16:24]]
        size = functools.reduce(jnp.add, [jnp.abs(b) for b in blk])
        return _cat(blk, 0), (l >= L_LO) & (l <= L_HI) & (size <= O_HI)

    def long_conv(c, cols):
        def spectrum(c):
            k = [_cat([yf_s[j, c, w, :, cols] for j in range(2)], 0) for w in range(3)]
            return k[0] - k[2], k[0] + k[1]

        (re0, im0), (re1, im1) = spectrum(c), spectrum(c + 1)
        re1, im1 = re1 - im0, im1 + re0
        if not isinstance(c, int):
            re, im = spectrum(jnp.maximum(c - 1, 0))
            re0, im0 = re0 - jnp.where(c > 0, im, 0.0), im0 + jnp.where(c > 0, re, 0.0)
        elif c:
            re, im = spectrum(c - 1)
            re0, im0 = re0 - im, im0 + re
        even = _dot(const_v[4 * C:4 * C + C // 2, :], _cat([re0, re1], 1))
        odd = _dot(const_v[4 * C + C // 2:5 * C, :], _cat([im0, im1], 1))
        back = even - odd
        y = _cat([even + odd] + [_flip8(back[r:r + 8]) for r in range(C // 2 - 8, -8, -8)], 0)
        return _cat([y[:, 0:128], y[:, 128:256]], 0)

    def mix(c, rows, o, pace, done):
        o = o.astype(BF16).T
        corner = _cat([_dot(o[_tile(r, 64), 512:D], wo_v[512:D, 512:D]) for r in range(4)], 0)
        edge = _cat([_dot(o[:, 512:D], wo_v[512:D, 0:512]), corner], 1)
        pace.after(edge)
        skip = d_v[...].astype(F32).reshape(1, D)
        for l in range(NL):
            cols = _tile(l)
            y = long_conv(c, cols)
            att = _dot(o[:, 0:512], wo_v[0:512, cols])
            pace.after(att)
            b = (y + kv_v[rows, cols].astype(F32) * skip[:, cols]) * x_v[rows, cols].astype(F32)
            g = gate_s[rows, :]
            out_v[rows, cols] = (g * (att + edge[:, cols]) + (1.0 - g) * b).astype(BF16)
            done(l)
        pace.flush()

    load_keep()
    st = {name: jnp.zeros((8, 128), F32) for name in ("bad", "q")}
    sent = []

    def norm_job(p, c, mark):
        st[p, c], ok = normalise(p, _tile(c), mark)
        st["bad"] = jnp.where(ok, st["bad"], 1.0)

    def size_job(p, c, mark):
        st["q"] = jnp.maximum(st["q"], pin(_peak(qv_s[p, c, 0:48, Q_LANES]), mark))

    def send(c, l):
        if c + 2 < NC:
            cols = {NL - 1: slice(None)}.get(l)
        else:
            cols = {NL - 2: pl.ds(0, D - 128), NL - 1: pl.ds(D - 128, 128)}.get(l)
        if cols is not None:
            sent.append(pltpu.make_async_copy(*part(out_v, out_hbm, (pl.ds(c * C, 2 * C), cols)), sems.at[0]))
            sent[-1].start()

    for p in range(NPAIR):
        for c in range(2):
            norm_job(p, c, None)
    for c in range(0, NC, 2):
        o = _cat([_cat([st.pop((p, j)) for p in range(NPAIR)], 0) for j in (c, c + 1)], 1)
        jobs = [(2, functools.partial(norm_job, p, j)) for p in range(NPAIR) for j in (c + 2, c + 3) if j < NC]
        jobs += [(1, functools.partial(size_job, p, j)) for p in range(NPAIR) for j in (c, c + 1)]
        mix(c, _tile(c // 2, 2 * C), o, _Pacer(jobs, 15 * sum(w for w, _ in jobs)), functools.partial(send, c))
    redo = (jnp.max(st["bad"]) > 0.0) | (jnp.max(st["q"]) * jnp.max(k_peak) > QK_HI)
    for c in sent:
        c.wait()

    @pl.when(redo)
    def _():
        @pl.loop(0, NPAIR * NC)
        def _(i):
            p, c = i // NC, i % NC
            for odd in range(2):
                w = qv_s[p, c, _tile(odd, 24), Q_LANES]
                s = _reverse_groups(_cat([scores(p, odd, t, w) for t in range(NC)], 0))
                e = jnp.exp2(s - jnp.max(s, axis=0, keepdims=True)) * (1.0 / S)
                ot_s[p + 1, _tile(odd, 24), pl.ds(pl.multiple_of(c * C, C), C)] = _dot(
                    _side_by_side(qv_s[p, :, _tile(odd, 24), V_LANES]), e)

        @pl.loop(0, NC // 2)
        def _(i):
            both = [pl.ds(pl.multiple_of((2 * i + j) * C, C), C) for j in range(2)]
            o = _cat([_cat([normalise(p, cols)[0] for p in range(NPAIR)], 0) for cols in both], 1)
            mix(2 * i, pl.ds(pl.multiple_of(2 * i * C, 2 * C), 2 * C), o, _Pacer([]), lambda l: None)

        everything = pltpu.make_async_copy(out_v, out_hbm, sems.at[0])
        everything.start()
        everything.wait()


@jax.jit
def pallas_gated_mix__mha_block__ssm_conv_h3__prompt_kernel(
    A_x: jax.Array,
    A_wqkv: jax.Array,
    A_wo: jax.Array,
    B_q: jax.Array,
    B_k: jax.Array,
    B_v: jax.Array,
    B_shift_k: jax.Array,
    B_ssm_k: jax.Array,
    B_ssm_D: jax.Array,
    gate_w: jax.Array,
):
    del B_q
    vm = pltpu.VMEM
    scratch = [
        [vm((NPAIR if b == len(BLOCKS) - 1 else 1, 10, 112, 128), F32) for b in range(len(BLOCKS))],
        vm((S, D), BF16), vm((D, D), BF16), vm((D, D), BF16), vm((D, D), BF16), vm((D, D), BF16),
        vm((S, D), BF16), vm((S, D), BF16), vm((D, S), BF16),
        vm((D, D), U32), vm((S // 2, D), U32), vm((NPAIR, 32, 4 * C * VPU_TILES), F32),
        vm((NPAIR, S // 2, 128), U32), vm((NPAIR, NC, 56, 384), F32), vm((NPAIR + 1, 48, S), F32),
        vm((C // 2 * len(LATE), TQ), U32),
        vm((2, NC, 2, C // 2, D), F32), vm((2, NC, 2, C // 2, D), F32), vm((2, NC, 3, C // 2, D), F32),
        vm((S, 128), F32),
        vm(_CONSTANTS.shape, BF16), vm((4, D), BF16), vm((D,), BF16), vm((D,), BF16),
        pltpu.SemaphoreType.DMA((len(K_STAGES) + len(KV_STAGES) + 2,)),
    ]
    hbm = pl.BlockSpec(memory_space=pltpu.HBM)
    out = pl.pallas_call(
        _kernel,
        out_shape=jax.ShapeDtypeStruct((S, D), BF16),
        in_specs=[hbm] * 10,
        out_specs=hbm,
        scratch_shapes=scratch,
        compiler_params=pltpu.CompilerParams(vmem_limit_bytes=127 * 2 ** 20),
    )(A_x.reshape(S, D), A_wqkv, A_wo, B_k.reshape(S, D), B_v.reshape(S, D), B_shift_k.T, B_ssm_k,
      B_ssm_D, gate_w, _CONSTANTS)
    return out.reshape(1, S, D)
```
